```python
import jax
import jax.numpy as jnp

def _softmax(x, axis=-1):
    return jax.nn.softmax(x, axis=axis)
def _gelu(x):
    return jax.nn.gelu(x, approximate=True)
def _silu(x):
    return jax.nn.silu(x)
def _sigmoid(x):
    return jax.nn.sigmoid(x)
def _layernorm(x, axis=-1, eps=1e-5):
    m = jnp.mean(x, axis=axis, keepdims=True)
    v = jnp.var(x, axis=axis, keepdims=True)
    return (x - m) / jnp.sqrt(v + eps)
def _scatter_add(tgt, idx, src, axis=0):
    return tgt.at[idx].add(src)
def _segment_sum(src, seg, n):
    return jax.ops.segment_sum(src, seg, n)
class _Rng:
    def __init__(self, key):
        self._k = key
    def _next(self):
        self._k, sub = jax.random.split(self._k)
        return sub
    def normal(self, shape):
        return jax.random.normal(self._next(), shape, dtype=jnp.bfloat16)
    def randint(self, lo, hi, shape):
        return jax.random.randint(self._next(), shape, lo, hi, dtype=jnp.int32)
    def uniform(self, shape, lo=0.0, hi=1.0):
        return jax.random.uniform(self._next(), shape, jnp.bfloat16, lo, hi)
    def permutation(self, n):
        return jax.random.permutation(self._next(), n)


kernel_name = 'gated_mix__compressed_kv_cla__moe_arch_mod__prompt'

def setup_inputs():
    _rng = _Rng(jax.random.key(int.from_bytes(__import__("os").urandom(4), "little")))
    _w = (lambda a: (lambda t: t.astype(jnp.bfloat16) if jnp.issubdtype(t.dtype, jnp.floating) else t)(jnp.asarray(a)))
    def _A_setup():
        B, H, Sq, Sk, D, M = 1, 16, 2048, 2048, 256, 448
        Dc = 4 * D
        return {
            "x": _w((lambda *s: _rng.normal(s) * 0.05)(B, Sq, M)),
            "c_kv": _w((lambda *s: _rng.normal(s) * 0.05)(B, Sk, Dc)),
            "w_q": _w((lambda *s: _rng.normal(s) * 0.05)(M, H, D) * (M ** -0.5)),
            "w_uk": _w((lambda *s: _rng.normal(s) * 0.05)(Dc, H, D) * (Dc ** -0.5)),
            "w_uv": _w((lambda *s: _rng.normal(s) * 0.05)(Dc, H, D) * (Dc ** -0.5)),
            "w_o": _w((lambda *s: _rng.normal(s) * 0.05)(H, D, M) * ((H * D) ** -0.5)),
        }
    _A_in = _A_setup()

    def _B_setup():
        B, S, D, F, C = 1, 2048, 448, 1792, 2
        return {
            "x": _w((lambda *s: _rng.normal(s) * 0.05)(B, S, D)),
            "w_r": _w((lambda *s: _rng.normal(s) * 0.05)(D)),
            "w_gate": _w((lambda *s: _rng.normal(s) * 0.05)(D, F)),
            "w_up": _w((lambda *s: _rng.normal(s) * 0.05)(D, F)),
            "w_down": _w((lambda *s: _rng.normal(s) * 0.05)(F, D)),
        }
    _B_in = _B_setup()

    return {
        "A_x": _A_in["x"],
        "A_c_kv": _A_in["c_kv"],
        "A_w_q": _A_in["w_q"],
        "A_w_uk": _A_in["w_uk"],
        "A_w_uv": _A_in["w_uv"],
        "A_w_o": _A_in["w_o"],
        "B_x": _B_in["x"],
        "B_w_r": _B_in["w_r"],
        "B_w_gate": _B_in["w_gate"],
        "B_w_up": _B_in["w_up"],
        "B_w_down": _B_in["w_down"],
        "gate_w": _w((lambda *s: _rng.normal(s) * 0.05)(448)),
    }

def reference(A_x, A_c_kv, A_w_q, A_w_uk, A_w_uv, A_w_o, B_x, B_w_r, B_w_gate, B_w_up, B_w_down, gate_w):
    def _A_ref(x, c_kv, w_q, w_uk, w_uv, w_o):
        B, Sq, M = x.shape[0], x.shape[1], x.shape[2]
        Sk = c_kv.shape[1]
        H, D = w_q.shape[1], w_q.shape[2]
        q = jnp.einsum("bqm,mhd->bhqd", x, w_q)
        k = jnp.einsum("bkc,chd->bhkd", c_kv, w_uk)
        v = jnp.einsum("bkc,chd->bhkd", c_kv, w_uv)
        scores = jnp.einsum("bhqd,bhkd->bhqk", q, k) * (D ** -0.5)
        off = Sk - Sq
        qi = jnp.arange(Sq)[:, None]
        kj = jnp.arange(Sk)[None, :]
        cmask = kj <= (qi + off)
        scores = jnp.where(cmask[None, None], scores, -1e9)
        p = _softmax(scores, axis=-1)
        ctx = jnp.einsum("bhqk,bhkd->bhqd", p, v)
        return jnp.einsum("bhqd,hdm->bqm", ctx, w_o)

    def _B_ref(x, w_r, w_gate, w_up, w_down):
        B, S, D = x.shape
        C = 2
        r = x @ w_r
        idx = jnp.argsort(-r, axis=-1)[:, :C]
        idx_e = jnp.repeat(idx.reshape(B, C, 1), D, axis=2)
        x_sel = jnp.take_along_axis(x, idx_e, axis=1)
        g = _silu(x_sel @ w_gate)
        u = x_sel @ w_up
        y = (g * u) @ w_down
        r_sel = _sigmoid(jnp.take_along_axis(r, idx, axis=1))
        y = y * r_sel.reshape(B, C, 1)
        b_off = (jnp.arange(B) * S).reshape(B, 1)
        flat_idx = (idx + b_off).reshape(B * C)
        zero = (x * 0.0).reshape(B * S, D)
        upd = _scatter_add(zero, flat_idx, y.reshape(B * C, D), axis=0)
        return x + upd.reshape(B, S, D)

    x = A_x
    g = _sigmoid((x * gate_w).sum(-1, keepdims=True))
    a = _A_ref(x, A_c_kv, A_w_q, A_w_uk, A_w_uv, A_w_o)
    b = _B_ref(x, B_w_r, B_w_gate, B_w_up, B_w_down)
    return g * a + (1 - g) * b
```

```python
import functools

import jax
import jax.numpy as jnp
import numpy as np
from jax import lax
import jax.experimental.pallas as pl
import jax.experimental.pallas.tpu as pltpu

F32 = jnp.float32
BF16 = jnp.bfloat16
NN = (((1,), (0,)), ((), ()))
NT = (((1,), (1,)), ((), ()))
LOG2E = 1.4426950408889634

CFG = dict(TB=256)


def _dot(a, b, dn=NN):
    return lax.dot_general(a, b, dn, preferred_element_type=F32)


def _kernel(xT_hbm, c_hbm, wq_hbm, wk_hbm, wv_hbm, woT_hbm, vec_ref, wg_hbm, wu_hbm, wdT_hbm,
            o_hbm,
            xT, c, wq32, wk32, wv32, woT, wg, wu, wdT,
            wqT, wk, wvT, qT, k, vT, sT, acc, obuf, rg, ycol,
            sem_in, sem_w, sem_o, *, H, S, D, M, DC):
    TB = CFG["TB"]
    NB = S // TB
    scale = float(D) ** -0.5 * LOG2E

    def w_copies(p, slot):
        return (
            pltpu.make_async_copy(wq_hbm.bitcast(jnp.uint32).at[:, p, :], wq32.at[slot], sem_w.at[slot, 0]),
            pltpu.make_async_copy(wk_hbm.bitcast(jnp.uint32).at[:, p, :], wk32.at[slot], sem_w.at[slot, 1]),
            pltpu.make_async_copy(wv_hbm.bitcast(jnp.uint32).at[:, p, :], wv32.at[slot], sem_w.at[slot, 2]),
            pltpu.make_async_copy(woT_hbm.at[pl.ds(2 * p, 2)], woT.at[slot], sem_w.at[slot, 3]),
        )

    cp_x = pltpu.make_async_copy(xT_hbm, xT, sem_in.at[0])
    cp_c = pltpu.make_async_copy(c_hbm, c, sem_in.at[1])
    cp_ffn = (
        pltpu.make_async_copy(wg_hbm, wg, sem_in.at[2]),
        pltpu.make_async_copy(wu_hbm, wu, sem_in.at[3]),
        pltpu.make_async_copy(wdT_hbm, wdT, sem_in.at[4]),
    )
    cp_x.start()
    for cp in w_copies(0, 0):
        cp.start()
    cp_c.start()
    for cp in cp_ffn:
        cp.start()

    acc[...] = jnp.zeros(acc.shape, F32)
    cp_x.wait()
    rg[...] = _dot(vec_ref[...], xT[...])
    cp_c.wait()

    def head(h, carry):
        p = h // 2
        slot = p % 2
        odd = h % 2

        @pl.when(odd == 0)
        def _():
            for cp in w_copies(p, slot):
                cp.wait()

            @pl.when(p + 1 < H // 2)
            def _():
                for cp in w_copies(p + 1, 1 - slot):
                    cp.start()

        sh = (16 * (1 - odd)).astype(jnp.uint32)

        def unpack(w32):
            return pltpu.bitcast((w32 << sh) & jnp.uint32(0xFFFF0000), F32)

        wk[...] = unpack(wk32[slot]).astype(BF16)
        wqT[...] = unpack(wq32[slot]).T.astype(BF16)
        wvT[...] = unpack(wv32[slot]).T.astype(BF16)

        def tok(j):
            return slice(j * TB, (j + 1) * TB)

        def kp(j):
            k[tok(j), :] = _dot(c[tok(j), :], wk[...]).astype(BF16)

        def qp(j):
            qT[:, tok(j)] = (_dot(wqT[...], xT[:, tok(j)]) * scale).astype(BF16)

        def vp(j):
            vT[:, tok(j)] = _dot(wvT[...], c[tok(j), :], NT).astype(BF16)

        tri = (lax.broadcasted_iota(jnp.int32, (128, 128), 0)
               <= lax.broadcasted_iota(jnp.int32, (128, 128), 1))
        mx = {}

        def qk(t):
            n = 128 * (t + 1)
            b = t % 4
            s = _dot(k[0:n, :], qT[:, 128 * t:128 * (t + 1)])
            sd = jnp.where(tri, s[n - 128:, :], -1e9 * LOG2E)
            m = jnp.max(sd, axis=0, keepdims=True)
            if t > 0:
                sT[b, 0:n - 128, :] = s[:n - 128, :]
                m = jnp.maximum(m, jnp.max(s[:n - 128, :], axis=0, keepdims=True))
            sT[b, n - 128:n, :] = sd
            mx[t] = m

        ot = {}

        def pv(t):
            n = 128 * (t + 1)
            b = t % 4
            e = jnp.exp2(sT[b, 0:n, :] - mx[t])
            l = jnp.sum(e, axis=0, keepdims=True)
            o = _dot(vT[:, 0:n], e.astype(BF16))
            ot[t] = (o * (1.0 / l)).astype(BF16)

        def op(j):
            r = TB // 128
            o = jnp.concatenate([ot[j * r + i] for i in range(r)], axis=1)
            acc[:, tok(j)] += _dot(woT[slot, odd], o)

        r = TB // 128
        for j in range(NB):
            kp(j)
            qp(j)
            vp(j)
            if j >= 2:
                op(j - 2)
            if j >= 1:
                for i in range(r):
                    pv((j - 1) * r + i)
            for i in range(r):
                qk(j * r + i)
        op(NB - 2)
        for i in range(r):
            pv((NB - 1) * r + i)
        op(NB - 1)
        return carry

    lax.fori_loop(0, H, head, 0)

    for cp in cp_ffn:
        cp.wait()
    rr = rg[0:1, :].astype(BF16).astype(F32)
    pos = lax.broadcasted_iota(jnp.int32, (1, S), 1)
    m1 = jnp.max(rr, axis=1, keepdims=True)
    i1 = jnp.min(jnp.where(rr == m1, pos, S), axis=1, keepdims=True)
    rr2 = jnp.where(pos == i1, -jnp.inf, rr)
    m2 = jnp.max(rr2, axis=1, keepdims=True)
    i2 = jnp.min(jnp.where((rr2 == m2) & (pos != i1), pos, S), axis=1, keepdims=True)
    row = lax.broadcasted_iota(jnp.int32, (16, S), 0)
    pos16 = lax.broadcasted_iota(jnp.int32, (16, S), 1)
    onehot = jnp.where(((row == 0) & (pos16 == i1)) | ((row == 1) & (pos16 == i2)), 1.0, 0.0).astype(BF16)
    xs = _dot(onehot, xT[...], NT).astype(BF16)
    gt = _dot(xs, wg[...])
    up = _dot(xs, wu[...])
    hh = (gt * jax.nn.sigmoid(gt) * up).astype(BF16)
    y = _dot(hh, wdT[...], NT)
    row1 = lax.broadcasted_iota(jnp.int32, (16, 1), 0)
    y = y * jax.nn.sigmoid(jnp.where(row1 == 0, m1, m2))
    ycol[...] = jnp.concatenate([y, jnp.zeros((112, M), F32)], axis=0).T

    for j in range(NB):
        sl = slice(j * TB, (j + 1) * TB)
        g = jax.nn.sigmoid(rg[1:2, sl])
        pj = pos[:, sl]
        upd = jnp.where(pj == i1, ycol[:, 0:1], jnp.where(pj == i2, ycol[:, 1:2], 0.0))
        b = xT[:, sl].astype(F32) + upd
        obuf[:, sl] = (g * acc[:, sl] + (1.0 - g) * b).astype(BF16)
    cp_o = pltpu.make_async_copy(obuf, o_hbm, sem_o)
    cp_o.start()
    cp_o.wait()


@jax.jit
def pallas_gated_mix__compressed_kv_cla__moe_arch_mod__prompt_kernel(A_x, A_c_kv, A_w_q, A_w_uk, A_w_uv, A_w_o, B_x, B_w_r, B_w_gate, B_w_up, B_w_down, gate_w):
    del B_x
    _, S, M = A_x.shape
    DC = A_c_kv.shape[2]
    _, H, D = A_w_q.shape
    F = B_w_gate.shape[1]
    xT = A_x[0].T
    c = A_c_kv[0]
    woT = jnp.transpose(A_w_o, (0, 2, 1))
    wdT = B_w_down.T
    vec = jnp.concatenate([B_w_r[None], gate_w[None], jnp.zeros((14, M), BF16)], axis=0)
    any_spec = pl.BlockSpec(memory_space=pl.ANY)
    outT = pl.pallas_call(
        functools.partial(_kernel, H=H, S=S, D=D, M=M, DC=DC),
        in_specs=[any_spec] * 6 + [pl.BlockSpec(memory_space=pltpu.VMEM)] + [any_spec] * 3,
        out_specs=any_spec,
        out_shape=jax.ShapeDtypeStruct((M, S), BF16),
        scratch_shapes=[
            pltpu.VMEM((M, S), BF16),
            pltpu.VMEM((S, DC), BF16),
            pltpu.VMEM((2, M, D), jnp.uint32),
            pltpu.VMEM((2, DC, D), jnp.uint32),
            pltpu.VMEM((2, DC, D), jnp.uint32),
            pltpu.VMEM((2, 2, M, D), BF16),
            pltpu.VMEM((M, F), BF16),
            pltpu.VMEM((M, F), BF16),
            pltpu.VMEM((M, F), BF16),
            pltpu.VMEM((D, M), BF16),
            pltpu.VMEM((DC, D), BF16),
            pltpu.VMEM((D, DC), BF16),
            pltpu.VMEM((D, S), BF16),
            pltpu.VMEM((S, D), BF16),
            pltpu.VMEM((D, S), BF16),
            pltpu.VMEM((4, S, 128), F32),
            pltpu.VMEM((M, S), F32),
            pltpu.VMEM((M, S), BF16),
            pltpu.VMEM((16, S), F32),
            pltpu.VMEM((M, 128), F32),
            pltpu.SemaphoreType.DMA((5,)),
            pltpu.SemaphoreType.DMA((2, 4)),
            pltpu.SemaphoreType.DMA,
        ],
        compiler_params=pltpu.CompilerParams(vmem_limit_bytes=100 * 2**20),
        name="gated_mix",
    )(xT, c, A_w_q, A_w_uk, A_w_uv, woT, vec, B_w_gate, B_w_up, wdT)
    return outT.T[None]
```

```python
import functools

import jax
import jax.numpy as jnp
import numpy as np
from jax import lax
import jax.experimental.pallas as pl
import jax.experimental.pallas.tpu as pltpu

F32 = jnp.float32
BF16 = jnp.bfloat16
U32 = jnp.uint32
NN = (((1,), (0,)), ((), ()))
NT = (((1,), (1,)), ((), ()))
LOG2E = 1.4426950408889634
TB = 256
NZ = 16

CFG = dict(QC=256, PC=512, ODMA=1, EARLY=0, TBF=1, PB=1, XS=(512,))


def _dot(a, b, dn=NN):
    return lax.dot_general(a, b, dn, preferred_element_type=F32)


def _red8(x, f):
    parts = [x[i:i + 8] for i in range(0, x.shape[0], 8)]
    while len(parts) > 1:
        parts = [f(parts[i], parts[i + 1]) if i + 1 < len(parts) else parts[i]
                 for i in range(0, len(parts), 2)]
    return parts[0]


def _lo(w32):
    return pltpu.bitcast(w32 << 16, F32)


def _hi(w32):
    return pltpu.bitcast(w32 & jnp.uint32(0xFFFF0000), F32)


def _kernel(xT_hbm, c_hbm, wq_hbm, wk_hbm, wv_hbm, woT_hbm, vec_ref, wg_hbm, wu_hbm, wdT_hbm,
            o_hbm,
            xT32, c32, wq32, wk32, wv32, woT32, wg32, wu32, wdT32,
            wqA32, wqB32, qT32, k32, vT32, oA32, oB32, sT, acc, ob, rg, zero,
            sem_x, sem_q, sem_in, sem_w, sem_o, *, H, S, D, M, DC):
    NB = S // TB
    NP = H // 2
    NF = wg32.shape[1] // 128
    scale = float(D) ** -0.5 * LOG2E
    xT, c, woT, wqA, wqB, qT, k, vT, oA, oB, wg, wu, wdT = (
        a.bitcast(BF16) for a in (
            xT32, c32, woT32, wqA32, wqB32, qT32, k32, vT32, oA32, oB32, wg32, wu32, wdT32))

    def tok(j):
        return slice(j * TB, (j + 1) * TB)

    XS = (0,) + tuple(CFG["XS"]) + (S,)
    cp_x = [pltpu.make_async_copy(xT_hbm.bitcast(U32).at[:, lo:hi], xT32.at[0, :, lo:hi], sem_x.at[i])
            for i, (lo, hi) in enumerate(zip(XS, XS[1:]))]
    cp_q = [pltpu.make_async_copy(wq_hbm.bitcast(U32).at[:, p, :], wq32.at[p], sem_q.at[p]) for p in range(NP)]
    cp_c = pltpu.make_async_copy(c_hbm.bitcast(U32), c32, sem_in.at[0])
    cp_ffn = (
        pltpu.make_async_copy(wg_hbm.bitcast(U32), wg32, sem_in.at[1]),
        pltpu.make_async_copy(wu_hbm.bitcast(U32), wu32, sem_in.at[2]),
        pltpu.make_async_copy(wdT_hbm.bitcast(U32), wdT32, sem_in.at[3]),
    )
    cp_wo = pltpu.make_async_copy(woT_hbm.bitcast(U32), woT32, sem_in.at[4])

    def w_copies(p, slot):
        return (
            pltpu.make_async_copy(wk_hbm.bitcast(U32).at[:, p, :], wk32.at[slot], sem_w.at[slot, 0]),
            pltpu.make_async_copy(wv_hbm.bitcast(U32).at[:, p, :], wv32.at[slot], sem_w.at[slot, 1]),
        )

    def o_copy(j):
        return pltpu.make_async_copy(ob.at[:, tok(j)], o_hbm.at[:, tok(j)], sem_o.at[j])

    cp_q[0].start()
    for cp in cp_x:
        cp.start()
    for p in range(1, 4):
        cp_q[p].start()

    def start_rest():
        for p in range(4, NP):
            cp_q[p].start()
        for cp in cp_ffn:
            cp.start()
        for cp in w_copies(0, 0):
            cp.start()
        cp_c.start()
        cp_wo.start()

    if CFG["EARLY"]:
        start_rest()

    @pl.loop(0, NZ)
    def _(i):
        zero[i] = 0

    def prep_q(p):
        wt = wq32[p].T
        (wqA, wqB)[p % 2][0, 0:D, :] = _lo(wt).astype(BF16)
        (wqA, wqB)[p % 2][0, D:2 * D, :] = _hi(wt).astype(BF16)

    def q_pair(p, j):
        w = (wqA, wqB)[p % 2][zero[j]]
        if p == 0:
            w = jnp.concatenate([w, vec_ref[...]], axis=0)
        v = lax.dot_general(w, xT[zero[p], :, tok(j)], NN, preferred_element_type=F32)
        if p == 0:
            rg[:, tok(j)] = v[2 * D:]
        v = (v[:2 * D] * scale).astype(BF16)
        qT[2 * p, :, tok(j)] = v[:D]
        qT[2 * p + 1, :, tok(j)] = v[D:]

    def route():
        rr = rg[0:1, :].astype(BF16).astype(F32)
        pos = lax.broadcasted_iota(jnp.int32, (1, S), 1)
        m1 = jnp.max(rr)
        i1 = jnp.min(jnp.where(rr == m1, pos, S))
        rr2 = jnp.where(pos == i1, -jnp.inf, rr)
        m2 = jnp.max(rr2)
        i2 = jnp.min(jnp.where((rr2 == m2) & (pos != i1), pos, S))
        return (i1, m1), (i2, m2)

    def tile_of(idx):
        return pl.ds(pl.multiple_of(jnp.clip(idx // 128, 0, S // 128 - 1) * 128, 128), 128)

    def gather(sel):
        row = lax.broadcasted_iota(jnp.int32, (16, 128), 0)
        lane = lax.broadcasted_iota(jnp.int32, (16, 128), 1)
        xs = None
        for n, (idx, _) in enumerate(sel):
            onehot = jnp.where((row == n) & (lane == idx % 128), 1.0, 0.0).astype(BF16)
            part = lax.dot_general(onehot, xT[0, :, tile_of(idx)], NT, preferred_element_type=F32)
            xs = part if xs is None else xs + part
        return xs.astype(BF16)

    def ffn_hidden(xs, i):
        f = slice(128 * i, 128 * (i + 1))
        gt = lax.dot_general(xs, wg[:, f], NN, preferred_element_type=F32)
        up = lax.dot_general(xs, wu[:, f], NN, preferred_element_type=F32)
        return (gt * jax.nn.sigmoid(gt) * up).astype(BF16)

    def ffn_down(hid, i):
        return lax.dot_general(hid, wdT[:, 128 * i:128 * (i + 1)], NT, preferred_element_type=F32)

    def scatter(sel, y):
        row = lax.broadcasted_iota(jnp.int32, (128, M), 0)
        for n, (idx, score) in enumerate(sel):
            yn = y[n:n + 1] * jax.nn.sigmoid(jnp.full((1, M), score))
            upd = jnp.where(row == idx % 128, yn, 0.0).T
            t = tile_of(idx)
            acc[0, :, t] += (1.0 - rg[2:3, t]) * upd

    def init_acc(j):
        g = jax.nn.sigmoid(rg[1:2, tok(j)])
        rg[2:3, tok(j)] = g
        acc[0, :, tok(j)] = (1.0 - g) * xT[zero[NZ - 1], :, tok(j)].astype(F32)

    cp_q[0].wait()
    cp_x[0].wait()
    prep_q(0)
    for p in range(NP):
        for j in range(NB):
            if p == 0 and j * TB in XS[1:]:
                cp_x[XS.index(j * TB)].wait()
                if j * TB == XS[-2]:
                    for pp in range(1, 4):
                        cp_q[pp].wait()
                    if not CFG["EARLY"]:
                        start_rest()
            if p == 3 and j == NB // 2:
                for pp in range(4, NP):
                    cp_q[pp].wait()
                for cp in cp_ffn:
                    cp.wait()
            q_pair(p, j)
            if j == NB - 3 and p + 1 < NP:
                prep_q(p + 1)
            if p == 1:
                init_acc(j)
            if p == 2 and j == 0:
                sel = route()
            if p == 3 and j == NB // 2:
                xs = gather(sel)
            step = (p - 3) * NB + j - NB // 2 - 1
            if 0 <= step < 2 * NF:
                if step % 2 == 0:
                    hid = ffn_hidden(xs, step // 2)
                else:
                    part = ffn_down(hid, step // 2)
                    y = part if step == 1 else y + part
            if step == 2 * NF:
                scatter(sel, y)
    cp_c.wait()
    cp_wo.wait()

    def head(h, carry):
        odd = h % 2
        p = h // 2
        slot = p % 2

        @pl.when(odd == 0)
        def _():
            for cp in w_copies(p, slot):
                cp.wait()

            @pl.when(p + 1 < NP)
            def _():
                for cp in w_copies(p + 1, 1 - slot):
                    cp.start()

        z = zero[0]
        sh = (16 * (1 - odd)).astype(U32)
        QC = CFG["QC"]
        PC = CFG["PC"]
        PB = CFG["PB"]

        def unpack(w32):
            return pltpu.bitcast((w32 << sh) & jnp.uint32(0xFFFF0000), F32).astype(BF16)

        def kp(j):
            if j % PB == 0:
                rows = slice(j * TB, (j + PB) * TB)
                k[0, rows, :] = lax.dot_general(c[rows, :], unpack(wk32[slot + zero[j]]), NN, preferred_element_type=F32).astype(BF16)

        def vp(j):
            if j % PB == 0:
                rows = slice(j * TB, (j + PB) * TB)
                v = lax.dot_general(c[rows, :], unpack(wv32[slot + zero[j]]), NN, preferred_element_type=F32)
                vT[0, :, rows] = v.astype(BF16).T if CFG["TBF"] else v.T.astype(BF16)

        tri = (lax.broadcasted_iota(jnp.int32, (128, 128), 0)
               <= lax.broadcasted_iota(jnp.int32, (128, 128), 1))
        mx = {}

        def qk(t):
            n = 128 * (t + 1)
            m = None
            for lo in range(0, n, QC):
                hi = min(lo + QC, n)
                s = lax.dot_general(k[z, lo:hi, :], qT[h, :, 128 * t:128 * (t + 1)], NN, preferred_element_type=F32)
                if hi == n:
                    sd = jnp.where(tri, s[hi - lo - 128:, :], -1e9 * LOG2E)
                    s = jnp.concatenate([s[:hi - lo - 128], sd], axis=0) if hi - lo > 128 else sd
                sT[t % 2, lo:hi, :] = s
                mc = _red8(s, jnp.maximum)
                m = mc if m is None else jnp.maximum(m, mc)
            mx[t] = jnp.max(m, axis=0, keepdims=True)

        def pv(t):
            n = 128 * (t + 1)
            l = o = None
            for lo in range(0, n, PC):
                hi = min(lo + PC, n)
                e = jnp.exp2(sT[t % 2 + z, lo:hi, :] - mx[t])
                lc = _red8(e, jnp.add)
                l = lc if l is None else l + lc
                oc = lax.dot_general(vT[z, :, lo:hi], e.astype(BF16), NN, preferred_element_type=F32)
                o = oc if o is None else o + oc
            w = rg[2:3, 128 * t:128 * (t + 1)] / jnp.sum(l, axis=0, keepdims=True)
            j = t // 2
            (oA, oB)[j % 2][0, :, 128 * (t % 4):128 * (t % 4 + 1)] = (o * w).astype(BF16)

        def op(j):
            o = (oA, oB)[j % 2][z, :, 128 * (2 * j % 4):128 * (2 * j % 4 + 2)]
            a = acc[0, :, tok(j)] + lax.dot_general(woT[h], o, NN, preferred_element_type=F32)
            acc[0, :, tok(j)] = a
            if CFG["ODMA"]:
                ob[:, tok(j)] = a.astype(BF16)

                @pl.when(h == H - 1)
                def _():
                    o_copy(j).start()

        kp(0)
        vp(0)
        qk(0)
        qk(1)
        for j in range(1, NB):
            kp(j)
            pv(2 * j - 2)
            pv(2 * j - 1)
            vp(j)
            qk(2 * j)
            qk(2 * j + 1)
            if j >= 2:
                op(j - 2)
        pv(2 * NB - 2)
        pv(2 * NB - 1)
        op(NB - 2)
        op(NB - 1)
        return carry

    lax.fori_loop(0, H, head, 0)

    if not CFG["ODMA"]:
        for j in range(NB):
            ob[:, tok(j)] = acc[0, :, tok(j)].astype(BF16)
            o_copy(j).start()
    for j in range(NB):
        o_copy(j).wait()


@jax.jit
def pallas_gated_mix__compressed_kv_cla__moe_arch_mod__prompt_kernel(A_x, A_c_kv, A_w_q, A_w_uk, A_w_uv, A_w_o, B_x, B_w_r, B_w_gate, B_w_up, B_w_down, gate_w):
    del B_x
    _, S, M = A_x.shape
    DC = A_c_kv.shape[2]
    _, H, D = A_w_q.shape
    F = B_w_gate.shape[1]
    xT = A_x[0].T
    c = A_c_kv[0]
    woT = jnp.transpose(A_w_o, (0, 2, 1))
    wdT = B_w_down.T
    vec = jnp.concatenate([B_w_r[None], gate_w[None], jnp.zeros((14, M), BF16)], axis=0)
    any_spec = pl.BlockSpec(memory_space=pl.ANY)
    outT = pl.pallas_call(
        functools.partial(_kernel, H=H, S=S, D=D, M=M, DC=DC),
        in_specs=[any_spec] * 6 + [pl.BlockSpec(memory_space=pltpu.VMEM)] + [any_spec] * 3,
        out_specs=any_spec,
        out_shape=jax.ShapeDtypeStruct((M, S), BF16),
        scratch_shapes=[
            pltpu.VMEM((1, M // 2, S), U32),
            pltpu.VMEM((S // 2, DC), U32),
            pltpu.VMEM((H // 2, M, D), U32),
            pltpu.VMEM((2, DC, D), U32),
            pltpu.VMEM((2, DC, D), U32),
            pltpu.VMEM((H, M // 2, D), U32),
            pltpu.VMEM((M // 2, F), U32),
            pltpu.VMEM((M // 2, F), U32),
            pltpu.VMEM((M // 2, F), U32),
            pltpu.VMEM((1, D, M), U32),
            pltpu.VMEM((1, D, M), U32),
            pltpu.VMEM((H, D // 2, S), U32),
            pltpu.VMEM((1, S // 2, D), U32),
            pltpu.VMEM((1, D // 2, S), U32),
            pltpu.VMEM((1, D // 2, 2 * TB), U32),
            pltpu.VMEM((1, D // 2, 2 * TB), U32),
            pltpu.VMEM((2, S, 128), F32),
            pltpu.VMEM((1, M, S), F32),
            pltpu.VMEM((M, S), BF16),
            pltpu.VMEM((16, S), F32),
            pltpu.SMEM((NZ,), jnp.int32),
            pltpu.SemaphoreType.DMA((len(CFG["XS"]) + 1,)),
            pltpu.SemaphoreType.DMA((H // 2,)),
            pltpu.SemaphoreType.DMA((5,)),
            pltpu.SemaphoreType.DMA((2, 2)),
            pltpu.SemaphoreType.DMA((S // TB,)),
        ],
        compiler_params=pltpu.CompilerParams(vmem_limit_bytes=100 * 2**20),
        name="gated_mix",
    )(xT, c, A_w_q, A_w_uk, A_w_uv, woT, vec, B_w_gate, B_w_up, wdT)
    return outT.T[None]
```

```python
import functools

import jax
import jax.numpy as jnp
from jax import lax
import jax.experimental.pallas as pl
import jax.experimental.pallas.tpu as pltpu

F32 = jnp.float32
BF16 = jnp.bfloat16
U32 = jnp.uint32
NN = (((1,), (0,)), ((), ()))
NT = (((1,), (1,)), ((), ()))
TN = (((0,), (0,)), ((), ()))
LOG2E = 1.4426950408889634
TB = 256
NZ = 16
NPQ = 3

CFG = dict(QC=256, PC=512, XS=(512, 1536), OSPLIT=1, QPOS=0, IS=65536, RP=0, W1=1, SC=1, C0=0, C1=5, FJ=2, DOQ=1, AL=7)


def _red8(x, f):
    parts = [x[i:i + 8] for i in range(0, x.shape[0], 8)]
    while len(parts) > 1:
        parts = [f(parts[i], parts[i + 1]) if i + 1 < len(parts) else parts[i]
                 for i in range(0, len(parts), 2)]
    return parts[0]


def _half(w32, sh):
    return pltpu.bitcast((w32 << sh) & jnp.uint32(0xFFFF0000), F32)


def _kernel(xT_hbm, c_hbm, wq_hbm, wk_hbm, wv_hbm, woT_hbm, wr_hbm, gw_hbm, wg_hbm, wu_hbm, wdT_hbm,
            o_hbm,
            xT32, c32, wq32, wk32, wv32, woT32, wg, wu, wdT, wr, gw, zrow,
            wqT32, qT32, k32, vT32, oA32, oB32, sT, acc, ob, rg, xs, ycur, zero, top,
            sem_x, sem_q, sem_in, sem_w, sem_o, *, H, S, D, M, F):
    NB = S // TB
    NP = H // 2
    NF = F // 128
    NU = (H - 2 * NPQ) * NB // H
    assert NU * H == (H - 2 * NPQ) * NB and NF < H
    scale = float(D) ** -0.5 * LOG2E
    xT, c, woT, wqT, qT, k, vT, oA, oB = (
        a.bitcast(BF16) for a in (xT32, c32, woT32, wqT32, qT32, k32, vT32, oA32, oB32))

    def tok(j):
        return slice(j * TB, (j + 1) * TB)

    XS = (0,) + tuple(CFG["XS"]) + (S,)
    cp_x = [pltpu.make_async_copy(xT_hbm.bitcast(U32).at[:, lo:hi], xT32.at[0, :, lo:hi], sem_x.at[i])
            for i, (lo, hi) in enumerate(zip(XS, XS[1:]))]
    cp_q = [pltpu.make_async_copy(wq_hbm.bitcast(U32).at[:, p, :], wq32.at[p], sem_q.at[p]) for p in range(NP)]
    cp_c = pltpu.make_async_copy(c_hbm.bitcast(U32), c32, sem_in.at[0])
    cp_wo = [pltpu.make_async_copy(woT_hbm.bitcast(U32).at[sl], woT32.at[sl], sem_in.at[1 + i])
             for i, sl in enumerate((pl.ds(0, 1), pl.ds(1, H - 1)))]
    cp_vec = (pltpu.make_async_copy(wr_hbm, wr, sem_in.at[3]),
              pltpu.make_async_copy(gw_hbm, gw, sem_in.at[4]))

    def w_copies(h):
        slot = h & 1
        f = pl.ds(pl.multiple_of(jnp.minimum(h, NF - 1) * 128, 128), 128)
        return (
            pltpu.make_async_copy(wk_hbm.bitcast(U32).at[:, h >> 1, :], wk32.at[slot], sem_w.at[slot, 0]),
            pltpu.make_async_copy(wv_hbm.bitcast(U32).at[:, h >> 1, :], wv32.at[slot], sem_w.at[slot, 1]),
            pltpu.make_async_copy(wg_hbm.at[:, f], wg.at[slot], sem_w.at[slot, 2]),
            pltpu.make_async_copy(wu_hbm.at[:, f], wu.at[slot], sem_w.at[slot, 3]),
            pltpu.make_async_copy(wdT_hbm.at[:, f], wdT.at[slot], sem_w.at[slot, 4]),
        )[CFG["C0"]:CFG["C1"]]

    def o_copy(j):
        return pltpu.make_async_copy(ob.at[:, tok(j)], o_hbm.at[:, tok(j)], sem_o.at[j])

    for cp in (cp_q[0], cp_x[0], *cp_vec, *cp_x[1:], *cp_q[1:NPQ + 1], cp_c, *w_copies(0), cp_wo[0],
               *cp_q[NPQ + 1:], cp_wo[1]):
        cp.start()

    @pl.loop(0, NZ)
    def _(i):
        zero[i] = 0

    def prep_q(p):
        wt = wq32[p].T
        wqT[p, 0:D, :] = _half(wt, 16).astype(BF16)
        wqT[p, D:2 * D, :] = _half(wt, 0).astype(BF16)

    def q_pair(p, j):
        w = wqT[p]
        if p == 0:
            w = jnp.concatenate([w, vec], axis=0)
        v = lax.dot_general(w, xT[zero[p], :, tok(j)], NN, preferred_element_type=F32)
        if p == 0:
            rg[0:1, tok(j)] = v[2 * D:2 * D + 1]
            rg[1:2, tok(j)] = jax.nn.sigmoid(v[2 * D + 1:2 * D + 2])
        qT[2 * p, :, tok(j)] = (v[:D] * scale).astype(BF16)
        qT[2 * p + 1, :, tok(j)] = (v[D:2 * D] * scale).astype(BF16)
        return v[0:1]

    def route():
        rr = rg[0:1, 0:S].astype(BF16).astype(F32)
        pos = lax.broadcasted_iota(jnp.int32, (1, S), 1).astype(F32)
        m1 = jnp.max(rr, axis=1, keepdims=True)
        i1 = jnp.min(jnp.where(rr == m1, pos, S - 1), axis=1, keepdims=True)
        rr2 = jnp.where(pos == i1, -jnp.inf, rr)
        m2 = jnp.max(rr2, axis=1, keepdims=True)
        i2 = jnp.min(jnp.where((rr2 == m2) & (pos != i1), pos, S - 1), axis=1, keepdims=True)
        return i1.astype(jnp.int32), i2.astype(jnp.int32)

    def init_acc(j, rows, after):
        keep = jnp.where(zero[NZ - 1] != 0, after, 1.0 - rg[1:2, tok(j)])
        acc[rows, tok(j)] = keep * xT[zero[NZ - 1], rows, tok(j)].astype(F32)

    def tile_of(idx):
        return pl.ds(pl.multiple_of(jnp.clip(idx >> 7, 0, S // 128 - 1) * 128, 128), 128)

    with jax.named_scope("wait0"):
        for cp in (cp_q[0], cp_x[0], *cp_vec):
            cp.wait()
    row = lax.broadcasted_iota(jnp.int32, (16, M), 0)
    vec = jnp.where(row == 0, wr[...].astype(F32).reshape(1, M),
                    jnp.where(row == 1, gw[...].astype(F32).reshape(1, M), 0.0)).astype(BF16)
    prep_q(0)
    for p in range(NPQ):
        for j in range(NB):
            if p == 0 and j * TB in XS[1:]:
                with jax.named_scope("wait1"):
                    cp_x[XS.index(j * TB)].wait()
                    if j * TB == XS[-2]:
                        for cp in cp_q[1:NPQ]:
                            cp.wait()
            last = q_pair(p, j)
            if j == NB - 2 and p + 1 < NPQ:
                prep_q(p + 1)
            if p == 1 and j == 0:
                sel = route()
            if p >= 1:
                init_acc(j, slice((p - 1) * M // (NPQ - 1), p * M // (NPQ - 1)), last)

    for n in range(2):
        top[n] = sel[n][0, 0]
    with jax.named_scope("wait3"):
        for cp in (cp_q[NPQ], cp_c, cp_wo[0]):
            cp.wait()
    part = []
    for n in range(2):
        onehot = jnp.where((lax.broadcasted_iota(jnp.int32, (16, 128), 0) == n)
                           & (lax.broadcasted_iota(jnp.int32, (16, 128), 1) == (top[n] & 127)), 1.0, 0.0)
        part.append(lax.dot_general(onehot.astype(BF16), xT[0, :, tile_of(top[n])], NT,
                                    preferred_element_type=F32))
    xs[...] = (part[0] + part[1]).astype(BF16)
    ycur[...] = jnp.zeros(ycur.shape, F32)
    zrow[...] = jnp.zeros(zrow.shape, F32)

    def head(h, carry):
        slot = h & 1

        if CFG["W1"]:
            @pl.when(h == 1)
            def _():
                for cp in (*cp_q[NPQ + 1:], cp_wo[1]):
                    cp.wait()

        @pl.loop(0, jnp.where(h == H - 1, 2, 0) if CFG['SC'] else 0)
        def _(n):
            t = tile_of(top[n])
            upd = jnp.where(lax.broadcasted_iota(jnp.int32, (128, M), 0) == (top[n] & 127),
                            ycur[pl.ds(n, 1), :], zrow[0]).T
            score = rg[0:1, t].astype(BF16).astype(F32)
            acc[:, t] += (1.0 - rg[1:2, t]) * jax.nn.sigmoid(score) * upd

        for cp in w_copies(h):
            cp.wait()

        @pl.when(h + 1 < H)
        def _():
            for cp in w_copies(h + 1):
                cp.start()

        z = zero[0]
        sh = (16 - 16 * slot).astype(U32)
        QC = CFG["QC"]
        PC = CFG["PC"]

        def qp(i):
            u = h * NU + i
            hq = 2 * NPQ + u // NB
            cols = pl.ds(pl.multiple_of((u % NB) * TB, TB), TB)
            w = _half(wq32[hq >> 1], (16 - 16 * (hq & 1)).astype(U32)).astype(BF16)
            v = lax.dot_general(w, xT[0, :, cols], TN, preferred_element_type=F32)
            qT[hq, :, cols] = (v * scale).astype(BF16)

        def kp(j):
            w = _half(wk32[slot + zero[j]], sh).astype(BF16)
            k[0, tok(j), :] = lax.dot_general(c[tok(j), :], w, NN, preferred_element_type=F32).astype(BF16)

        def vp(j):
            w = _half(wv32[slot + zero[j]], sh).astype(BF16)
            vT[0, :, tok(j)] = lax.dot_general(c[tok(j), :], w, NN, preferred_element_type=F32).astype(BF16).T

        def ffn_hidden():
            gt = lax.dot_general(xs[...], wg[slot], NN, preferred_element_type=F32)
            up = lax.dot_general(xs[...], wu[slot], NN, preferred_element_type=F32)
            return (gt * jax.nn.sigmoid(gt) * up).astype(BF16)

        def ffn_down(hid):
            y = lax.dot_general(hid, wdT[slot], NT, preferred_element_type=F32)
            ycur[...] += jnp.where(h < NF, y, 0.0)

        tri = (lax.broadcasted_iota(jnp.int32, (128, 128), 0)
               <= lax.broadcasted_iota(jnp.int32, (128, 128), 1))
        mx = {}

        def qk(t):
            n = 128 * (t + 1)
            m = None
            for lo in range(0, n, QC):
                hi = min(lo + QC, n)
                s = lax.dot_general(k[z, lo:hi, :], qT[h, :, 128 * t:128 * (t + 1)], NN, preferred_element_type=F32)
                if hi == n:
                    sd = jnp.where(tri, s[hi - lo - 128:, :], -1e9 * LOG2E)
                    s = jnp.concatenate([s[:hi - lo - 128], sd], axis=0) if hi - lo > 128 else sd
                sT[t % 2, lo:hi, :] = s
                mc = _red8(s, jnp.maximum)
                m = mc if m is None else jnp.maximum(m, mc)
            mx[t] = jnp.max(m, axis=0, keepdims=True)

        def pv(t):
            n = 128 * (t + 1)
            l = o = None
            for lo in range(0, n, PC):
                hi = min(lo + PC, n)
                e = jnp.exp2(sT[t % 2 + z, lo:hi, :] - mx[t])
                lc = _red8(e, jnp.add)
                l = lc if l is None else l + lc
                oc = lax.dot_general(vT[z, :, lo:hi], e.astype(BF16), NN, preferred_element_type=F32)
                o = oc if o is None else o + oc
            w = rg[1:2, 128 * t:128 * (t + 1)] / jnp.sum(l, axis=0, keepdims=True)
            (oA, oB)[t // 2 % 2][0, :, 128 * (t % 4):128 * (t % 4 + 1)] = (o * w).astype(BF16)

        def op(j, parts=1):
            o = (oA, oB)[j % 2][z, :, 128 * (2 * j % 4):128 * (2 * j % 4 + 2)]
            for i in range(parts):
                rows = slice(i * M // parts, (i + 1) * M // parts)
                a = acc[rows, tok(j)] + lax.dot_general(woT[h, rows, :], o, NN, preferred_element_type=F32)
                acc[rows, tok(j)] = a
                ob[rows, tok(j)] = a.astype(BF16)

            @pl.when(h == H - 1)
            def _():
                o_copy(j).start()

        kp(0)
        for i in range(NU * CFG['DOQ']):
            qp(i)
        vp(0)
        qk(0)
        qk(1)
        for j in range(1, NB):
            kp(j)
            if j == CFG['FJ']:
                hid = ffn_hidden()
            pv(2 * j - 2)
            pv(2 * j - 1)
            vp(j)
            if j == CFG['FJ']:
                ffn_down(hid)
            qk(2 * j)
            qk(2 * j + 1)
            if j >= 2:
                op(j - 2)
        pv(2 * NB - 2)
        pv(2 * NB - 1)
        op(NB - 2, 1 + CFG["OSPLIT"])
        op(NB - 1)
        return carry

    lax.fori_loop(0, H, head, 0)
    if not CFG["W1"]:
        for cp in (*cp_q[NPQ + 1:], cp_wo[1]):
            cp.wait()

    with jax.named_scope("tail"):
        for j in range(NB):
            o_copy(j).wait()


@jax.jit
def pallas_gated_mix__compressed_kv_cla__moe_arch_mod__prompt_kernel(A_x, A_c_kv, A_w_q, A_w_uk, A_w_uv, A_w_o, B_x, B_w_r, B_w_gate, B_w_up, B_w_down, gate_w):
    del B_x
    _, S, M = A_x.shape
    DC = A_c_kv.shape[2]
    _, H, D = A_w_q.shape
    F = B_w_gate.shape[1]
    any_spec = pl.BlockSpec(memory_space=pl.ANY)
    outT = pl.pallas_call(
        functools.partial(_kernel, H=H, S=S, D=D, M=M, F=F),
        in_specs=[any_spec] * 11,
        out_specs=any_spec,
        out_shape=jax.ShapeDtypeStruct((M, S), BF16),
        scratch_shapes=[
            pltpu.VMEM((1, M // 2, S), U32),
            pltpu.VMEM((S // 2, DC), U32),
            pltpu.VMEM((H // 2, M, D), U32),
            pltpu.VMEM((2, DC, D), U32),
            pltpu.VMEM((2, DC, D), U32),
            pltpu.VMEM((H, M // 2, D), U32),
            pltpu.VMEM((2, M, 128), BF16),
            pltpu.VMEM((2, M, 128), BF16),
            pltpu.VMEM((2, M, 128), BF16),
            pltpu.VMEM((M,), BF16),
            pltpu.VMEM((M,), BF16),
            pltpu.VMEM((CFG['AL'], 1, M), F32),
            pltpu.VMEM((NPQ, D, M), U32),
            pltpu.VMEM((H, D // 2, S), U32),
            pltpu.VMEM((1, S // 2, D), U32),
            pltpu.VMEM((1, D // 2, S), U32),
            pltpu.VMEM((1, D // 2, 2 * TB), U32),
            pltpu.VMEM((1, D // 2, 2 * TB), U32),
            pltpu.VMEM((2, S, 128), F32),
            pltpu.VMEM((M, S), F32),
            pltpu.VMEM((M, S), BF16),
            pltpu.VMEM((8, S + CFG['RP']), F32),
            pltpu.VMEM((16, M), BF16),
            pltpu.VMEM((16, M), F32),
            pltpu.SMEM((NZ,), jnp.int32),
            pltpu.SMEM((2,), jnp.int32),
            pltpu.SemaphoreType.DMA((len(CFG["XS"]) + 1,)),
            pltpu.SemaphoreType.DMA((H // 2,)),
            pltpu.SemaphoreType.DMA((5,)),
            pltpu.SemaphoreType.DMA((2, 5)),
            pltpu.SemaphoreType.DMA((S // TB,)),
        ],
        compiler_params=pltpu.CompilerParams(vmem_limit_bytes=100 * 2**20, internal_scratch_in_bytes=CFG['IS']),
        name="gated_mix",
    )(A_x[0].T, A_c_kv[0], A_w_q, A_w_uk, A_w_uv, jnp.transpose(A_w_o, (0, 2, 1)),
      B_w_r, gate_w, B_w_gate, B_w_up, B_w_down.T)
    return outT.T[None]
```

```python
import functools

import jax
import jax.numpy as jnp
from jax import lax
import jax.experimental.pallas as pl
import jax.experimental.pallas.tpu as pltpu

F32 = jnp.float32
BF16 = jnp.bfloat16
U32 = jnp.uint32
NN = (((1,), (0,)), ((), ()))
NT = (((1,), (1,)), ((), ()))
TN = (((0,), (0,)), ((), ()))
LOG2E = 1.4426950408889634
TB = 256
NZ = 16
NPQ = 3

CFG = dict(QC=256, PC=512, XS=(512, 1536), OSPLIT=1, LAG=4, NOBC=False, IS=65536, RP=0, W1=1, SC=1, C0=0, C1=5, FJ=2, DOQ=1, AL=7)


def _red8(x, f):
    parts = [x[i:i + 8] for i in range(0, x.shape[0], 8)]
    while len(parts) > 1:
        parts = [f(parts[i], parts[i + 1]) if i + 1 < len(parts) else parts[i]
                 for i in range(0, len(parts), 2)]
    return parts[0]


def _half(w32, sh):
    return pltpu.bitcast((w32 >> sh).astype(jnp.uint16), BF16)


def _kernel(xT_hbm, c_hbm, wq_hbm, wk_hbm, wv_hbm, woT_hbm, wr_hbm, gw_hbm, wg_hbm, wu_hbm, wdT_hbm,
            o_hbm,
            xT32, c32, wq32, wk32, wv32, woT32, wg, wu, wdT, wr, gw, zrow,
            wqT32, qT32, k32, vT32, o0, o1, o2, o3, sT, acc, ob, rg, xs, ycur, zero, top,
            sem_x, sem_q, sem_in, sem_w, sem_f, sem_o, *, H, S, D, M, F):
    NB = S // TB
    NP = H // 2
    NF = F // 128
    NU = (H - 2 * NPQ) * NB // H
    assert NU * H == (H - 2 * NPQ) * NB and NF < H
    scale = float(D) ** -0.5 * LOG2E
    xT, c, woT, wqT, qT, k, vT, *oT = (
        a.bitcast(BF16) for a in (xT32, c32, woT32, wqT32, qT32, k32, vT32, o0, o1, o2, o3))

    def tok(j):
        return slice(j * TB, (j + 1) * TB)

    XS = (0,) + tuple(CFG["XS"]) + (S,)
    cp_x = [pltpu.make_async_copy(xT_hbm.bitcast(U32).at[:, lo:hi], xT32.at[0, :, lo:hi], sem_x.at[i])
            for i, (lo, hi) in enumerate(zip(XS, XS[1:]))]
    cp_q = [pltpu.make_async_copy(wq_hbm.bitcast(U32).at[:, p, :], wq32.at[p], sem_q.at[p]) for p in range(NP)]
    cp_c = pltpu.make_async_copy(c_hbm.bitcast(U32), c32, sem_in.at[0])
    cp_wo = [pltpu.make_async_copy(woT_hbm.bitcast(U32).at[sl], woT32.at[sl], sem_in.at[1 + i])
             for i, sl in enumerate((pl.ds(0, 1), pl.ds(1, H - 1)))]
    cp_vec = (pltpu.make_async_copy(wr_hbm, wr, sem_in.at[3]),
              pltpu.make_async_copy(gw_hbm, gw, sem_in.at[4]))

    def kv_copies(p):
        return (pltpu.make_async_copy(wk_hbm.bitcast(U32).at[:, p, :], wk32.at[p], sem_w.at[0, p]),
                pltpu.make_async_copy(wv_hbm.bitcast(U32).at[:, p, :], wv32.at[p], sem_w.at[1, p]))

    cp_ffn = [[pltpu.make_async_copy(src.at[:, sl], dst.at[:, sl], sem_f.at[i, n])
               for n, (src, dst) in enumerate(((wg_hbm, wg), (wu_hbm, wu), (wdT_hbm, wdT)))]
              for i, sl in enumerate((pl.ds(0, 128), pl.ds(128, F - 128)))]

    def o_copy(j):
        return pltpu.make_async_copy(ob.at[:, tok(j)], o_hbm.at[:, tok(j)], sem_o.at[j])

    first = (cp_q[NPQ], cp_c, *kv_copies(0), cp_wo[0], *cp_ffn[0])
    second = (*cp_q[NPQ + 1:], cp_wo[1], *cp_ffn[1])
    for cp in (cp_q[0], cp_x[0], *cp_vec, *cp_x[1:], *cp_q[1:NPQ], *first):
        cp.start()

    @pl.loop(0, NZ)
    def _(i):
        zero[i] = 0

    def prep_q(p):
        wt = wq32[p].T
        wqT[p, 0:D, :] = _half(wt, 0)
        wqT[p, D:2 * D, :] = _half(wt, 16)

    def q_pair(p, j):
        w = wqT[p]
        if p == 0:
            w = jnp.concatenate([w, vec], axis=0)
        v = lax.dot_general(w, xT[zero[p], :, tok(j)], NN, preferred_element_type=F32)
        if p == 0:
            rg[0:1, tok(j)] = v[2 * D:2 * D + 1]
            rg[1:2, tok(j)] = jax.nn.sigmoid(v[2 * D + 1:2 * D + 2])
        qT[2 * p, :, tok(j)] = (v[:D] * scale).astype(BF16)
        qT[2 * p + 1, :, tok(j)] = (v[D:2 * D] * scale).astype(BF16)
        return v[0:1]

    def route():
        rr = rg[0:1, 0:S].astype(BF16).astype(F32)
        pos = lax.broadcasted_iota(jnp.int32, (1, S), 1).astype(F32)
        m1 = jnp.max(rr, axis=1, keepdims=True)
        i1 = jnp.min(jnp.where(rr == m1, pos, S - 1), axis=1, keepdims=True)
        rr2 = jnp.where(pos == i1, -jnp.inf, rr)
        m2 = jnp.max(rr2, axis=1, keepdims=True)
        i2 = jnp.min(jnp.where((rr2 == m2) & (pos != i1), pos, S - 1), axis=1, keepdims=True)
        return i1.astype(jnp.int32), i2.astype(jnp.int32)

    def init_acc(j, rows, after):
        keep = jnp.where(zero[NZ - 1] != 0, after, 1.0 - rg[1:2, tok(j)])
        acc[rows, tok(j)] = keep * xT[zero[NZ - 1], rows, tok(j)].astype(F32)

    def tile_of(idx):
        return pl.ds(pl.multiple_of(jnp.clip(idx >> 7, 0, S // 128 - 1) * 128, 128), 128)

    with jax.named_scope("wait0"):
        for cp in (cp_q[0], cp_x[0], *cp_vec):
            cp.wait()
    row = lax.broadcasted_iota(jnp.int32, (16, M), 0)
    vec = jnp.where(row == 0, wr[...].astype(F32).reshape(1, M),
                    jnp.where(row == 1, gw[...].astype(F32).reshape(1, M), 0.0)).astype(BF16)
    prep_q(0)
    for p in range(NPQ):
        for j in range(NB):
            if p == 0 and j * TB in XS[1:]:
                with jax.named_scope("wait1"):
                    cp_x[XS.index(j * TB)].wait()
                    if j * TB == XS[-2]:
                        for cp in cp_q[1:NPQ]:
                            cp.wait()
                        for cp in second:
                            cp.start()
            last = q_pair(p, j)
            if j == NB - 2 and p + 1 < NPQ:
                prep_q(p + 1)
            if p == 1 and j == 0:
                sel = route()
            if p >= 1:
                init_acc(j, slice((p - 1) * M // (NPQ - 1), p * M // (NPQ - 1)), last)

    for n in range(2):
        top[n] = sel[n][0, 0]
    with jax.named_scope("wait3"):
        for cp in first:
            cp.wait()
    part = []
    for n in range(2):
        onehot = jnp.where((lax.broadcasted_iota(jnp.int32, (16, 128), 0) == n)
                           & (lax.broadcasted_iota(jnp.int32, (16, 128), 1) == (top[n] & 127)), 1.0, 0.0)
        part.append(lax.dot_general(onehot.astype(BF16), xT[0, :, tile_of(top[n])], NT,
                                    preferred_element_type=F32))
    xs[...] = (part[0] + part[1]).astype(BF16)
    ycur[...] = jnp.zeros(ycur.shape, F32)
    zrow[...] = jnp.zeros(zrow.shape, F32)

    def head(h, carry):
        pair = h >> 1

        @pl.loop(0, h & 1)
        def _(_):
            @pl.when(h == 1)
            def _():
                for cp in second:
                    cp.wait()

            @pl.when(pair + 1 < NP)
            def _():
                for cp in kv_copies(pair + 1):
                    cp.start()

            @pl.loop(0, jnp.where(h == H - 1, 2, 0))
            def _(n):
                t = tile_of(top[n])
                upd = jnp.where(lax.broadcasted_iota(jnp.int32, (128, M), 0) == (top[n] & 127),
                                ycur[pl.ds(n, 1), :], zrow[0]).T
                score = rg[0:1, t].astype(BF16).astype(F32)
                acc[:, t] += (1.0 - rg[1:2, t]) * jax.nn.sigmoid(score) * upd

        @pl.when((h > 0) & ((h & 1) == 0))
        def _():
            for cp in kv_copies(pair):
                cp.wait()

        z = zero[0]
        sh = (16 * (h & 1)).astype(U32)
        fcol = pl.ds(pl.multiple_of(jnp.minimum(h, NF - 1) * 128, 128), 128)
        QC = CFG["QC"]
        PC = CFG["PC"]

        def qp(i):
            u = h * NU + i
            hq = 2 * NPQ + lax.div(u, NB)
            cols = pl.ds(pl.multiple_of(lax.rem(u, NB) * TB, TB), TB)
            w = _half(wq32[hq >> 1], (16 * (hq & 1)).astype(U32))
            v = lax.dot_general(w, xT[0, :, cols], TN, preferred_element_type=F32)
            qT[hq, :, cols] = (v * scale).astype(BF16)

        def kp(j):
            w = _half(wk32[pair + zero[j]], sh)
            k[0, tok(j), :] = lax.dot_general(c[tok(j), :], w, NN, preferred_element_type=F32).astype(BF16)

        def vp(j):
            w = _half(wv32[pair + zero[j]], sh)
            vT[0, :, tok(j)] = lax.dot_general(c[tok(j), :], w, NN, preferred_element_type=F32).astype(BF16).T

        def ffn_in(w):
            return lax.dot_general(xs[...], w[:, fcol], NN, preferred_element_type=F32)

        def ffn_out(gt, up):
            hid = (gt * jax.nn.sigmoid(gt) * up).astype(BF16)
            y = lax.dot_general(hid, wdT[:, fcol], NT, preferred_element_type=F32)
            ycur[...] += jnp.where(h < NF, y, 0.0)

        tri = (lax.broadcasted_iota(jnp.int32, (128, 128), 0)
               <= lax.broadcasted_iota(jnp.int32, (128, 128), 1))
        mx = {}

        def qk(t):
            n = 128 * (t + 1)
            m = None
            for lo in range(0, n, QC):
                hi = min(lo + QC, n)
                s = lax.dot_general(k[z, lo:hi, :], qT[h, :, 128 * t:128 * (t + 1)], NN, preferred_element_type=F32)
                if hi == n:
                    sd = jnp.where(tri, s[hi - lo - 128:, :], -1e9 * LOG2E)
                    s = jnp.concatenate([s[:hi - lo - 128], sd], axis=0) if hi - lo > 128 else sd
                sT[t % 2, lo:hi, :] = s
                mc = _red8(s, jnp.maximum)
                m = mc if m is None else jnp.maximum(m, mc)
            mx[t] = jnp.max(m, axis=0, keepdims=True)

        def pv(t):
            n = 128 * (t + 1)
            l = o = None
            for lo in range(0, n, PC):
                hi = min(lo + PC, n)
                e = jnp.exp2(sT[t % 2 + z, lo:hi, :] - mx[t])
                lc = _red8(e, jnp.add)
                l = lc if l is None else l + lc
                oc = lax.dot_general(vT[z, :, lo:hi], e.astype(BF16), NN, preferred_element_type=F32)
                o = oc if o is None else o + oc
            w = rg[1:2, 128 * t:128 * (t + 1)] / jnp.sum(l, axis=0, keepdims=True)
            oT[t // 2 % 4][0, :, 128 * (t % 2):128 * (t % 2 + 1)] = (o * w).astype(BF16)

        def op(j, parts=1):
            o = oT[j % 4][z]
            for i in range(parts):
                rows = slice(i * M // parts, (i + 1) * M // parts)
                a = acc[rows, tok(j)] + lax.dot_general(woT[h, rows, :], o, NN, preferred_element_type=F32)
                acc[rows, tok(j)] = a
                ob[rows, tok(j)] = a.astype(BF16)

            @pl.when(h == H - 1)
            def _():
                o_copy(j).start()

        LAG = CFG["LAG"]
        kp(0)
        qp(0)
        gt = ffn_in(wg)
        qp(1)
        up = ffn_in(wu)
        qp(2)
        qp(3)
        ffn_out(gt, up)
        qp(4)
        vp(0)
        qk(0)
        qk(1)
        for j in range(1, NB):
            kp(j)
            pv(2 * j - 2)
            pv(2 * j - 1)
            vp(j)
            qk(2 * j)
            qk(2 * j + 1)
            if j >= LAG:
                op(j - LAG)
        pv(2 * NB - 2)
        pv(2 * NB - 1)
        for j in range(NB - LAG, NB):
            op(j)
        return carry

    lax.fori_loop(0, H, head, 0)

    with jax.named_scope("tail"):
        for j in range(NB):
            o_copy(j).wait()


@jax.jit
def pallas_gated_mix__compressed_kv_cla__moe_arch_mod__prompt_kernel(A_x, A_c_kv, A_w_q, A_w_uk, A_w_uv, A_w_o, B_x, B_w_r, B_w_gate, B_w_up, B_w_down, gate_w):
    del B_x
    _, S, M = A_x.shape
    DC = A_c_kv.shape[2]
    _, H, D = A_w_q.shape
    F = B_w_gate.shape[1]
    any_spec = pl.BlockSpec(memory_space=pl.ANY)
    outT = pl.pallas_call(
        functools.partial(_kernel, H=H, S=S, D=D, M=M, F=F),
        in_specs=[any_spec] * 11,
        out_specs=any_spec,
        out_shape=jax.ShapeDtypeStruct((M, S), BF16),
        scratch_shapes=[
            pltpu.VMEM((1, M // 2, S), U32),
            pltpu.VMEM((S // 2, DC), U32),
            pltpu.VMEM((H // 2, M, D), U32),
            pltpu.VMEM((H // 2, DC, D), U32),
            pltpu.VMEM((H // 2, DC, D), U32),
            pltpu.VMEM((H, M // 2, D), U32),
            pltpu.VMEM((M, F), BF16),
            pltpu.VMEM((M, F), BF16),
            pltpu.VMEM((M, F), BF16),
            pltpu.VMEM((M,), BF16),
            pltpu.VMEM((M,), BF16),
            pltpu.VMEM((CFG['AL'], 1, M), F32),
            pltpu.VMEM((NPQ, D, M), U32),
            pltpu.VMEM((H, D // 2, S), U32),
            pltpu.VMEM((1, S // 2, D), U32),
            pltpu.VMEM((1, D // 2, S), U32),
            *[pltpu.VMEM((1, D // 2, TB), U32)] * 4,
            pltpu.VMEM((2, S, 128), F32),
            pltpu.VMEM((M, S), F32),
            pltpu.VMEM((M, S), BF16),
            pltpu.VMEM((8, S + CFG['RP']), F32),
            pltpu.VMEM((16, M), BF16),
            pltpu.VMEM((16, M), F32),
            pltpu.SMEM((NZ,), jnp.int32),
            pltpu.SMEM((2,), jnp.int32),
            pltpu.SemaphoreType.DMA((len(CFG["XS"]) + 1,)),
            pltpu.SemaphoreType.DMA((H // 2,)),
            pltpu.SemaphoreType.DMA((5,)),
            pltpu.SemaphoreType.DMA((2, H // 2)),
            pltpu.SemaphoreType.DMA((2, 3)),
            pltpu.SemaphoreType.DMA((S // TB,)),
        ],
        compiler_params=pltpu.CompilerParams(vmem_limit_bytes=100 * 2**20, internal_scratch_in_bytes=CFG['IS'], disable_bounds_checks=CFG['NOBC']),
        name="gated_mix",
    )(A_x[0].T, A_c_kv[0], A_w_q, A_w_uk, A_w_uv, jnp.transpose(A_w_o, (0, 2, 1)),
      B_w_r, gate_w, B_w_gate, B_w_up, B_w_down.T)
    return outT.T[None]
```

```python
import functools

import jax
import jax.numpy as jnp
from jax import lax
import jax.experimental.pallas as pl
import jax.experimental.pallas.tpu as pltpu

F32 = jnp.float32
BF16 = jnp.bfloat16
U32 = jnp.uint32
NN = (((1,), (0,)), ((), ()))
NT = (((1,), (1,)), ((), ()))
TN = (((0,), (0,)), ((), ()))
LOG2E = 1.4426950408889634
TB = 256
NZ = 16
NPQ = 3

CFG = dict(QC=256, PC=512, XS=(256, 768, 1536), OSPLIT=1, LAG=5, PK=1, E=(5, 9), NS=2, NOBC=False, IS=65536, RP=0, W1=1, SC=1, C0=0, C1=5, FJ=2, DOQ=1, AL=7)


def _red8(x, f):
    parts = [x[i:i + 8] for i in range(0, x.shape[0], 8)]
    while len(parts) > 1:
        parts = [f(parts[i], parts[i + 1]) if i + 1 < len(parts) else parts[i]
                 for i in range(0, len(parts), 2)]
    return parts[0]


def _half(w32, sh):
    return pltpu.bitcast((w32 >> sh).astype(jnp.uint16), BF16)


def _kernel(xT_hbm, c_hbm, wq_hbm, wk_hbm, wv_hbm, woT_hbm, wr_hbm, gw_hbm, wg_hbm, wu_hbm, wdT_hbm,
            o_hbm,
            xT32, c32, wq32, wk32, wv32, woT32, wg, wu, wdT, wr, gw, zrow,
            wqT32, qT32, k32, vT32, o32, sT, acc, ob, rg, xs, ycur, zero, top,
            sem, *, H, S, D, M, F):
    NB = S // TB
    NP = H // 2
    NF = F // 128
    NU = (H - 2 * NPQ) * NB // H
    assert NU * H == (H - 2 * NPQ) * NB and NF < H
    scale = float(D) ** -0.5 * LOG2E
    xT, c, woT, wqT, qT, k, vT, *oT = (
        a.bitcast(BF16) for a in (xT32, c32, woT32, wqT32, qT32, k32, vT32, *o32))

    def tok(j):
        return slice(j * TB, (j + 1) * TB)

    SEM_X = 4
    XS = (0,) + tuple(CFG["XS"]) + (S,)
    cp_x = [pltpu.make_async_copy(xT_hbm.bitcast(U32).at[:, lo:hi], xT32.at[0, :, lo:hi], sem.at[SEM_X + i])
            for i, (lo, hi) in enumerate(zip(XS, XS[1:]))]
    SEM_FIRST, SEM_SECOND, SEM_KV, SEM_OUT = range(4)
    cp_q = [pltpu.make_async_copy(
        wq_hbm.bitcast(U32).at[:, p, :], wq32.at[p],
        sem.at[SEM_X if p == 0 else SEM_X + len(XS) - 2 if p < NPQ else SEM_FIRST if p == NPQ else SEM_SECOND])
        for p in range(NP)]
    cp_c = pltpu.make_async_copy(c_hbm.bitcast(U32), c32, sem.at[SEM_FIRST])
    cp_wo = [pltpu.make_async_copy(woT_hbm.bitcast(U32).at[sl], woT32.at[sl], sem.at[SEM_FIRST + i])
             for i, sl in enumerate((pl.ds(0, 1), pl.ds(1, H - 1)))]
    cp_vec = (pltpu.make_async_copy(wr_hbm, wr, sem.at[SEM_X]),
              pltpu.make_async_copy(gw_hbm, gw, sem.at[SEM_X]))

    def kv_copies(p, s=2):
        return (pltpu.make_async_copy(wk_hbm.bitcast(U32).at[:, p, :], wk32.at[p], sem.at[s]),
                pltpu.make_async_copy(wv_hbm.bitcast(U32).at[:, p, :], wv32.at[p], sem.at[s]))

    cp_ffn = [[pltpu.make_async_copy(src.at[:, sl], dst.at[:, sl], sem.at[SEM_FIRST + i])
               for n, (src, dst) in enumerate(((wg_hbm, wg), (wu_hbm, wu), (wdT_hbm, wdT)))]
              for i, sl in enumerate((pl.ds(0, 128), pl.ds(128, F - 128)))]

    def o_copy(j):
        return pltpu.make_async_copy(ob.at[:, tok(j)], o_hbm.at[:, tok(j)], sem.at[SEM_OUT])

    first = (cp_q[NPQ], cp_c, *kv_copies(0, SEM_FIRST), cp_wo[0], *cp_ffn[0])
    second = (*cp_q[NPQ + 1:], cp_wo[1], *cp_ffn[1])
    early = [cp_q[0], cp_x[0], *cp_vec, *cp_x[1:], *cp_q[1:NPQ], *first]
    E0, E1 = CFG["E"]
    for cp in early[:E0]:
        cp.start()

    @pl.loop(0, NZ)
    def _(i):
        zero[i] = 0

    def prep_q(p):
        wt = wq32[p].T
        wqT[p, 0:D, :] = _half(wt, 0)
        wqT[p, D:2 * D, :] = _half(wt, 16)

    def q_pair(p, j):
        w = wqT[p]
        if p == 0:
            w = jnp.concatenate([w, vec], axis=0)
        v = lax.dot_general(w, xT[zero[p], :, tok(j)], NN, preferred_element_type=F32)
        if p == 0:
            rg[0:1, tok(j)] = v[2 * D:2 * D + 1]
            rg[1:2, tok(j)] = jax.nn.sigmoid(v[2 * D + 1:2 * D + 2])
        qT[2 * p, :, tok(j)] = (v[:D] * scale).astype(BF16)
        qT[2 * p + 1, :, tok(j)] = (v[D:2 * D] * scale).astype(BF16)
        return v[0:1]

    def route():
        rr = rg[0:1, 0:S].astype(BF16).astype(F32)
        pos = lax.broadcasted_iota(jnp.int32, (1, S), 1).astype(F32)
        m1 = jnp.max(rr, axis=1, keepdims=True)
        i1 = jnp.min(jnp.where(rr == m1, pos, S - 1), axis=1, keepdims=True)
        rr2 = jnp.where(pos == i1, -jnp.inf, rr)
        m2 = jnp.max(rr2, axis=1, keepdims=True)
        i2 = jnp.min(jnp.where((rr2 == m2) & (pos != i1), pos, S - 1), axis=1, keepdims=True)
        return i1.astype(jnp.int32), i2.astype(jnp.int32)

    def init_acc(j, rows, after):
        keep = jnp.where(zero[NZ - 1] != 0, after, 1.0 - rg[1:2, tok(j)])
        acc[rows, tok(j)] = keep * xT[zero[NZ - 1], rows, tok(j)].astype(F32)

    def gather(n, idx):
        lane = lax.broadcasted_iota(jnp.int32, (1, 128), 1)
        xw = jnp.zeros((M // 2, 128), U32)
        for t in range(S // 128):
            xw = jnp.where(lane + 128 * t == idx, xT32[zero[NZ - 2 - n], :, 128 * t:128 * (t + 1)], xw)
        pick = jnp.where(lax.broadcasted_iota(jnp.int32, (16, 128), 0) == n, 1.0, 0.0).astype(BF16)
        return lax.dot_general(pick, pltpu.bitcast(xw, BF16), NT, preferred_element_type=F32)

    def tile_of(idx):
        return pl.ds(pl.multiple_of(jnp.clip(idx >> 7, 0, S // 128 - 1) * 128, 128), 128)

    with jax.named_scope("wait0"):
        for cp in (cp_q[0], cp_x[0], *cp_vec):
            cp.wait()
    for cp in early[E0:E1]:
        cp.start()
    row = lax.broadcasted_iota(jnp.int32, (16, M), 0)
    vec = jnp.where(row == 0, wr[...].astype(F32).reshape(1, M),
                    jnp.where(row == 1, gw[...].astype(F32).reshape(1, M), 0.0)).astype(BF16)
    prep_q(0)
    for p in range(NPQ):
        for j in range(NB):
            if p == 0 and j * TB in XS[1:]:
                with jax.named_scope("wait1"):
                    if j * TB == XS[1]:
                        for cp in early[E1:]:
                            cp.start()
                    cp_x[XS.index(j * TB)].wait()
                    if j * TB == XS[-2]:
                        for cp in cp_q[1:NPQ]:
                            cp.wait()
                        for cp in second:
                            cp.start()
            last = q_pair(p, j)
            if j == NB - 2 and p + 1 < NPQ:
                prep_q(p + 1)
            if p == 1 and j == 0:
                sel = route()
            if p == NPQ - 1 and j == 2:
                x0 = gather(0, sel[0])
            if p == NPQ - 1 and j == 4:
                xs[...] = (x0 + gather(1, sel[1])).astype(BF16)
            if p >= 1:
                init_acc(j, slice((p - 1) * M // (NPQ - 1), p * M // (NPQ - 1)), last)

    for n in range(2):
        top[n] = sel[n][0, 0]
    zrow[...] = jnp.zeros(zrow.shape, F32)
    ycur[...] = jnp.zeros(ycur.shape, F32)
    with jax.named_scope("wait3"):
        for cp in first:
            cp.wait()

    def head(h, carry):
        pair = h >> 1

        @pl.loop(0, h & 1)
        def _(_):
            @pl.when(h == 1)
            def _():
                for cp in second:
                    cp.wait()

            @pl.when(pair + 1 < NP)
            def _():
                for cp in kv_copies(pair + 1):
                    cp.start()

            @pl.loop(0, jnp.where(h == H - 1, 1, 0))
            def _(_):
                lane = lax.broadcasted_iota(jnp.int32, (1, 128), 1)
                if CFG["PK"]:
                    w = pltpu.bitcast(ycur[...].astype(BF16), U32)[0:1]
                    w = jnp.broadcast_to(w, (128, M)).T
                for n in range(2):
                    t = tile_of(top[n])
                    if CFG["PK"]:
                        col = pltpu.bitcast((w >> (16 * n)) << 16, F32)
                    else:
                        col = jnp.broadcast_to(ycur[n:n + 1, :], (128, M)).T
                    score = rg[0:1, t].astype(BF16).astype(F32)
                    wgt = (1.0 - rg[1:2, t]) * jax.nn.sigmoid(score)
                    acc[:, t] += jnp.where(lane == (top[n] & 127), wgt * col, zrow[0, :, 0:128])

        @pl.when((h > 0) & ((h & 1) == 0))
        def _():
            for cp in kv_copies(pair):
                cp.wait()

        z = zero[0]
        sh = (16 * (h & 1)).astype(U32)
        fcol = pl.ds(pl.multiple_of(jnp.minimum(h, NF - 1) * 128, 128), 128)
        QC = CFG["QC"]
        PC = CFG["PC"]

        def qp(i):
            u = h * NU + i
            hq = 2 * NPQ + lax.div(u, NB)
            cols = pl.ds(pl.multiple_of(lax.rem(u, NB) * TB, TB), TB)
            w = _half(wq32[hq >> 1], (16 * (hq & 1)).astype(U32))
            v = lax.dot_general(w, xT[0, :, cols], TN, preferred_element_type=F32)
            qT[hq, :, cols] = (v * scale).astype(BF16)

        def kp(j):
            w = _half(wk32[pair + zero[j] if j else pair], sh)
            k[0, tok(j), :] = lax.dot_general(c[tok(j), :], w, NN, preferred_element_type=F32).astype(BF16)

        def vp(j):
            w = _half(wv32[pair + zero[j]], sh)
            vT[0, :, tok(j)] = lax.dot_general(c[tok(j), :], w, NN, preferred_element_type=F32).astype(BF16).T

        def ffn_in(w):
            return lax.dot_general(xs[...], w[:, fcol], NN, preferred_element_type=F32)

        def ffn_out(gt, up):
            hid = (gt * jax.nn.sigmoid(gt) * up).astype(BF16)
            y = lax.dot_general(hid, wdT[:, fcol], NT, preferred_element_type=F32)
            ycur[...] += jnp.where(h < NF, y, 0.0)

        tri = (lax.broadcasted_iota(jnp.int32, (128, 128), 0)
               <= lax.broadcasted_iota(jnp.int32, (128, 128), 1))
        mx = {}

        def qk(t):
            n = 128 * (t + 1)
            m = None
            for lo in range(0, n, QC):
                hi = min(lo + QC, n)
                s = lax.dot_general(k[z, lo:hi, :], qT[h, :, 128 * t:128 * (t + 1)], NN, preferred_element_type=F32)
                if hi == n:
                    sd = jnp.where(tri, s[hi - lo - 128:, :], -1e9 * LOG2E)
                    s = jnp.concatenate([s[:hi - lo - 128], sd], axis=0) if hi - lo > 128 else sd
                sT[t % len(sT)][0, lo:hi, :] = s
                mc = _red8(s, jnp.maximum)
                m = mc if m is None else jnp.maximum(m, mc)
            mx[t] = jnp.max(m, axis=0, keepdims=True)

        def pv(t):
            n = 128 * (t + 1)
            l = o = None
            for lo in range(0, n, PC):
                hi = min(lo + PC, n)
                e = jnp.exp2(sT[t % len(sT)][z, lo:hi, :] - mx[t])
                lc = _red8(e, jnp.add)
                l = lc if l is None else l + lc
                oc = lax.dot_general(vT[z, :, lo:hi], e.astype(BF16), NN, preferred_element_type=F32)
                o = oc if o is None else o + oc
            w = rg[1:2, 128 * t:128 * (t + 1)] / jnp.sum(l, axis=0, keepdims=True)
            oT[t // 2][0, :, 128 * (t % 2):128 * (t % 2 + 1)] = (o * w).astype(BF16)

        def op(j, parts=1):
            o = oT[j][z]
            for i in range(parts):
                rows = slice(i * M // parts, (i + 1) * M // parts)
                a = acc[rows, tok(j)] + lax.dot_general(woT[h, rows, :], o, NN, preferred_element_type=F32)
                acc[rows, tok(j)] = a
                ob[rows, tok(j)] = a.astype(BF16)

            @pl.when(h == H - 1)
            def _():
                o_copy(j).start()

        LAG = CFG["LAG"]
        kp(0)
        qp(0)
        gt = ffn_in(wg)
        qp(1)
        up = ffn_in(wu)
        qp(2)
        qp(3)
        ffn_out(gt, up)
        qp(4)
        vp(0)
        qk(0)
        qk(1)
        for j in range(1, NB):
            kp(j)
            pv(2 * j - 2)
            pv(2 * j - 1)
            vp(j)
            qk(2 * j)
            qk(2 * j + 1)
            if j >= LAG:
                op(j - LAG)
        pv(2 * NB - 2)
        pv(2 * NB - 1)
        for j in range(NB - LAG, NB):
            op(j)
        return carry

    lax.fori_loop(0, H, head, 0)

    with jax.named_scope("tail"):
        for j in range(NB):
            o_copy(j).wait()


@jax.jit
def pallas_gated_mix__compressed_kv_cla__moe_arch_mod__prompt_kernel(A_x, A_c_kv, A_w_q, A_w_uk, A_w_uv, A_w_o, B_x, B_w_r, B_w_gate, B_w_up, B_w_down, gate_w):
    del B_x
    _, S, M = A_x.shape
    DC = A_c_kv.shape[2]
    _, H, D = A_w_q.shape
    F = B_w_gate.shape[1]
    any_spec = pl.BlockSpec(memory_space=pl.ANY)
    outT = pl.pallas_call(
        functools.partial(_kernel, H=H, S=S, D=D, M=M, F=F),
        in_specs=[any_spec] * 11,
        out_specs=any_spec,
        out_shape=jax.ShapeDtypeStruct((M, S), BF16),
        scratch_shapes=[
            pltpu.VMEM((1, M // 2, S), U32),
            pltpu.VMEM((S // 2, DC), U32),
            pltpu.VMEM((H // 2, M, D), U32),
            pltpu.VMEM((H // 2, DC, D), U32),
            pltpu.VMEM((H // 2, DC, D), U32),
            pltpu.VMEM((H, M // 2, D), U32),
            pltpu.VMEM((M, F), BF16),
            pltpu.VMEM((M, F), BF16),
            pltpu.VMEM((M, F), BF16),
            pltpu.VMEM((M,), BF16),
            pltpu.VMEM((M,), BF16),
            pltpu.VMEM((CFG['AL'], 1, M), F32),
            pltpu.VMEM((NPQ, D, M), U32),
            pltpu.VMEM((H, D // 2, S), U32),
            pltpu.VMEM((1, S // 2, D), U32),
            pltpu.VMEM((1, D // 2, S), U32),
            [pltpu.VMEM((1, D // 2, TB), U32)] * (S // TB),
            [pltpu.VMEM((1, S, 128), F32)] * CFG['NS'],
            pltpu.VMEM((M, S), F32),
            pltpu.VMEM((M, S), BF16),
            pltpu.VMEM((8, S + CFG['RP']), F32),
            pltpu.VMEM((16, M), BF16),
            pltpu.VMEM((16, M), F32),
            pltpu.SMEM((NZ,), jnp.int32),
            pltpu.SMEM((2,), jnp.int32),
            pltpu.SemaphoreType.DMA((len(CFG["XS"]) + 5,)),
        ],
        compiler_params=pltpu.CompilerParams(vmem_limit_bytes=100 * 2**20, internal_scratch_in_bytes=CFG['IS'], disable_bounds_checks=CFG['NOBC']),
        name="gated_mix",
    )(A_x[0].T, A_c_kv[0], A_w_q, A_w_uk, A_w_uv, jnp.transpose(A_w_o, (0, 2, 1)),
      B_w_r, gate_w, B_w_gate, B_w_up, B_w_down.T)
    return outT.T[None]
```

```python
import functools

import jax
import jax.numpy as jnp
from jax import lax
import jax.experimental.pallas as pl
import jax.experimental.pallas.tpu as pltpu

F32 = jnp.float32
BF16 = jnp.bfloat16
U32 = jnp.uint32
I32 = jnp.int32
NN = (((1,), (0,)), ((), ()))
NT = (((1,), (1,)), ((), ()))
TN = (((0,), (0,)), ((), ()))
LOG2E = 1.4426950408889634
MASKED = -1e9 * LOG2E

TB = 256
NPQ = 3
X_SPLITS = (256, 1024)
OUT_LAG = 4
NZ = 16
SEM_FIRST, SEM_SECOND, SEM_KV, SEM_OUT, SEM_X = range(5)


def _dot(a, b, dims):
    return lax.dot_general(a, b, dims, preferred_element_type=F32)


def _fold8(x, f):
    parts = [x[i:i + 8] for i in range(0, x.shape[0], 8)]
    while len(parts) > 1:
        parts = [f(parts[i], parts[i + 1]) if i + 1 < len(parts) else parts[i]
                 for i in range(0, len(parts), 2)]
    return parts[0]


def _head(words, odd):
    shift = jnp.asarray(16 * odd).astype(U32)
    return pltpu.bitcast((words >> shift).astype(jnp.uint16), BF16)


def _kernel(xT_hbm, c_hbm, wq_hbm, wk_hbm, wv_hbm, woT_hbm, wr_hbm, gw_hbm, wg_hbm, wu_hbm, wdT_hbm,
            out_hbm,
            xT32, c32, wq32, wk32, wv32, woT32, wg, wu, wdT, wr, gw, zrow,
            wqT32, qT32, k32, vT32, oT32, sT, acc, out, rg, xsel, ysel, zero, top, sem,
            *, H, S, D, M, F):
    NB = S // TB
    NP = H // 2
    NF = F // 128
    NU = (H - 2 * NPQ) * NB // H
    assert NU * H == (H - 2 * NPQ) * NB and NU == 5 and NF < H
    q_scale = float(D) ** -0.5 * LOG2E
    xT, c, woT, wqT, qT, k, vT, *oT = (
        ref.bitcast(BF16) for ref in (xT32, c32, woT32, wqT32, qT32, k32, vT32, *oT32))

    def blk(j):
        return slice(j * TB, (j + 1) * TB)

    def tile(t):
        return slice(t * 128, (t + 1) * 128)

    def wq_copy(p, s):
        return pltpu.make_async_copy(wq_hbm.bitcast(U32).at[:, p, :], wq32.at[p], sem.at[s])

    def kv_copies(p, s):
        return [pltpu.make_async_copy(src.bitcast(U32).at[:, p, :], dst.at[p], sem.at[s])
                for src, dst in ((wk_hbm, wk32), (wv_hbm, wv32))]

    def wo_ffn_copies(heads, cols, s):
        return [pltpu.make_async_copy(woT_hbm.bitcast(U32).at[heads], woT32.at[heads], sem.at[s])] + [
            pltpu.make_async_copy(src.at[:, cols], dst.at[:, cols], sem.at[s])
            for src, dst in ((wg_hbm, wg), (wu_hbm, wu), (wdT_hbm, wdT))]

    def out_copy(j):
        return pltpu.make_async_copy(out.at[:, blk(j)], out_hbm.at[:, blk(j)], sem.at[SEM_OUT])

    edges = (0, *X_SPLITS, S)
    x_copy = [pltpu.make_async_copy(xT_hbm.bitcast(U32).at[:, lo:hi], xT32.at[0, :, lo:hi], sem.at[SEM_X + i])
              for i, (lo, hi) in enumerate(zip(edges, edges[1:]))]
    stage0 = [wq_copy(0, SEM_X), x_copy[0],
              pltpu.make_async_copy(wr_hbm, wr, sem.at[SEM_X]),
              pltpu.make_async_copy(gw_hbm, gw, sem.at[SEM_X])]
    stage1 = [x_copy[1]]
    stage2 = [x_copy[2]] + [wq_copy(p, SEM_X + 2) for p in range(1, NPQ)]
    step0 = ([wq_copy(NPQ, SEM_FIRST), pltpu.make_async_copy(c_hbm.bitcast(U32), c32, sem.at[SEM_FIRST])]
             + kv_copies(0, SEM_FIRST) + wo_ffn_copies(pl.ds(0, 1), pl.ds(0, 128), SEM_FIRST))
    step1 = ([wq_copy(p, SEM_SECOND) for p in range(NPQ + 1, NP)]
             + wo_ffn_copies(pl.ds(1, H - 1), pl.ds(128, F - 128), SEM_SECOND))

    def start(copies):
        for cp in copies:
            cp.start()

    def wait(copies):
        for cp in copies:
            cp.wait()

    start(stage0 + stage1)

    @pl.loop(0, NZ)
    def _(i):
        zero[i] = 0

    def transpose_wq(p):
        wqT[p, 0:D, :] = _head(wq32[p], 0).T
        wqT[p, D:2 * D, :] = _head(wq32[p], 1).T

    def project_q_pair(p, j):
        w = wqT[p]
        if p == 0:
            w = jnp.concatenate([w, vectors], axis=0)
        v = _dot(w, xT[zero[p], :, blk(j)], NN)
        if p == 0:
            rg[0:1, blk(j)] = v[2 * D:2 * D + 1].astype(BF16).astype(F32)
            rg[1:2, blk(j)] = jax.nn.sigmoid(v[2 * D + 1:2 * D + 2])
        qT[2 * p, :, blk(j)] = (v[:D] * q_scale).astype(BF16)
        qT[2 * p + 1, :, blk(j)] = (v[D:2 * D] * q_scale).astype(BF16)
        return v[0:1]

    def route():
        pos = lax.broadcasted_iota(I32, (1, S), 1).astype(F32)
        r1 = rg[0:1, :]
        i1 = jnp.min(jnp.where(r1 == jnp.max(r1, axis=1, keepdims=True), pos, S - 1), axis=1, keepdims=True)
        r2 = jnp.where(pos == i1, -jnp.inf, r1)
        hit = (r2 == jnp.max(r2, axis=1, keepdims=True)) & (pos != i1)
        i2 = jnp.min(jnp.where(hit, pos, S - 1), axis=1, keepdims=True)
        return i1.astype(I32), i2.astype(I32)

    def gather(n, idx):
        lane = lax.broadcasted_iota(I32, (1, 128), 1)
        words = jnp.zeros((M // 2, 128), U32)
        for t in range(S // 128):
            words = jnp.where(lane + 128 * t == idx, xT32[zero[NZ - 2 - n], :, tile(t)], words)
        pick = jnp.where(lax.broadcasted_iota(I32, (16, 128), 0) == n, 1.0, 0.0).astype(BF16)
        return _dot(pick, pltpu.bitcast(words, BF16), NT)

    def init_acc(j, rows, after):
        keep = jnp.where(zero[NZ - 1] != 0, after, 1.0 - rg[1:2, blk(j)])
        acc[rows, blk(j)] = keep * xT[zero[NZ - 1], rows, blk(j)].astype(F32)

    wait(stage0)
    start(stage2 + step0[:1])
    row = lax.broadcasted_iota(I32, (16, M), 0)
    vectors = jnp.where(row == 0, wr[...].astype(F32).reshape(1, M),
                        jnp.where(row == 1, gw[...].astype(F32).reshape(1, M), 0.0)).astype(BF16)
    transpose_wq(0)
    for p in range(NPQ):
        for j in range(NB):
            if p == 0 and j * TB == X_SPLITS[0]:
                start(step0[1:])
                wait(stage1)
            if p == 0 and j * TB == X_SPLITS[1]:
                wait(stage2)
                start(step1)
            latest = project_q_pair(p, j)
            if j == NB - 2 and p + 1 < NPQ:
                transpose_wq(p + 1)
            if p == 1 and j == 0:
                routed = route()
            if p == NPQ - 1 and j == 2:
                x_first = gather(0, routed[0])
            if p == NPQ - 1 and j == 4:
                xsel[...] = (x_first + gather(1, routed[1])).astype(BF16)
            if p >= 1:
                init_acc(j, slice((p - 1) * M // (NPQ - 1), p * M // (NPQ - 1)), latest)
    for n in range(2):
        top[n] = routed[n][0, 0]
    zrow[...] = jnp.zeros(zrow.shape, F32)
    ysel[...] = jnp.zeros(ysel.shape, F32)
    wait(step0)

    def head_step(h, carry):
        pair = h >> 1
        odd = h & 1
        lane = lax.broadcasted_iota(I32, (1, 128), 1)

        @pl.loop(0, odd)
        def _(_):
            @pl.when(h == 1)
            def _():
                wait(step1)

            @pl.when(pair + 1 < NP)
            def _():
                start(kv_copies(pair + 1, SEM_KV))

            @pl.loop(0, jnp.where(h == H - 1, 1, 0))
            def _(_):
                words = pltpu.bitcast(ysel[...].astype(BF16), U32)[0:1]
                words = jnp.broadcast_to(words, (128, M)).T
                for n in range(2):
                    cols = pl.ds(pl.multiple_of(jnp.clip(top[n] >> 7, 0, S // 128 - 1) * 128, 128), 128)
                    y = pltpu.bitcast((words >> (16 * n)) << 16, F32)
                    weight = (1.0 - rg[1:2, cols]) * jax.nn.sigmoid(rg[0:1, cols])
                    acc[:, cols] += jnp.where(lane == (top[n] & 127), weight * y, zrow[0, :, 0:128])

        @pl.when((h > 0) & (odd == 0))
        def _():
            wait(kv_copies(pair, SEM_KV))

        z = zero[0]

        def project_q(i):
            u = h * NU + i
            hq = 2 * NPQ + lax.div(u, NB)
            cols = pl.ds(pl.multiple_of(lax.rem(u, NB) * TB, TB), TB)
            v = _dot(_head(wq32[hq >> 1], hq & 1), xT[0, :, cols], TN)
            qT[hq, :, cols] = (v * q_scale).astype(BF16)

        def project_k(j):
            w = _head(wk32[pair + zero[j] if j else pair], odd)
            k[0, blk(j), :] = _dot(c[blk(j), :], w, NN).astype(BF16)

        def project_v(j):
            w = _head(wv32[pair + zero[j]], odd)
            vT[0, :, blk(j)] = _dot(c[blk(j), :], w, NN).astype(BF16).T

        hidden = pl.ds(pl.multiple_of(jnp.minimum(h, NF - 1) * 128, 128), 128)

        def ffn_in(w):
            return _dot(xsel[...], w[:, hidden], NN)

        def ffn_out(gate, up):
            y = _dot((gate * jax.nn.sigmoid(gate) * up).astype(BF16), wdT[:, hidden], NT)
            ysel[...] += jnp.where(h < NF, y, 0.0)

        causal = lax.broadcasted_iota(I32, (128, 128), 0) <= lax.broadcasted_iota(I32, (128, 128), 1)
        row_max = {}

        def keys(lo, hi):
            return k[z, lo:hi, :]

        def diagonal(j):
            base = j * TB
            kk = jnp.concatenate([keys(base + 64, base + 128), keys(base + 192, base + 256)], axis=0)
            late = _dot(qT[h, :, tile(2 * j + 1)].T[64:], kk, NT)
            late = jnp.concatenate([jnp.zeros((64, 128), F32), late], axis=0).T
            q = jnp.where(lane >= 64, qT32[h, :, tile(2 * j)], qT32[h, :, tile(2 * j + 1)])
            middle = _dot(keys(base + 64, base + 128), pltpu.bitcast(q, BF16), NN)
            return middle, late

        def scores(t, middle, late):
            base = t // 2 * TB
            q = qT[h, :, tile(t)]
            folded = []

            def put(lo, s):
                sT[t % 2][0, lo:lo + s.shape[0], :] = s
                m = _fold8(s, jnp.maximum)
                folded[:] = [jnp.maximum(folded[0], m) if folded else m]

            for lo in range(0, base, TB):
                put(lo, _dot(keys(lo, lo + TB), q, NN))
            if t % 2 == 0:
                put(base, jnp.where(causal[:64], _dot(keys(base, base + 64), q, NN), MASKED))
                put(base + 64, jnp.where(causal[64:], middle, MASKED))
            else:
                s = _dot(jnp.concatenate([keys(base, base + 64), keys(base + 128, base + 192)], axis=0), q, NN)
                put(base, s[:64])
                put(base + 64, jnp.where(lane < 64, middle, late[:64]))
                put(base + 128, jnp.where(causal[:64], s[64:], MASKED))
                put(base + 192, jnp.where(causal[64:], late[64:], MASKED))
            row_max[t] = jnp.max(folded[0], axis=0, keepdims=True)

        def context(t):
            total = ctx = None
            for i in range(t + 1):
                e = jnp.exp2(sT[t % 2][z, tile(i), :] - row_max[t])
                part = _fold8(e, jnp.add)
                total = part if total is None else total + part
                part = _dot(vT[z, :, tile(i)], e.astype(BF16), NN)
                ctx = part if ctx is None else ctx + part
            scale = rg[1:2, tile(t)] / jnp.sum(total, axis=0, keepdims=True)
            oT[t // 2][0, :, tile(t % 2)] = (ctx * scale).astype(BF16)

        def project_out(j):
            a = acc[:, blk(j)] + _dot(woT[h], oT[j][z], NN)
            acc[:, blk(j)] = a
            out[:, blk(j)] = a.astype(BF16)

            @pl.when(h == H - 1)
            def _():
                out_copy(j).start()

        project_k(0)
        project_q(0)
        gate = ffn_in(wg)
        project_q(1)
        up = ffn_in(wu)
        project_q(2)
        project_q(3)
        ffn_out(gate, up)
        project_q(4)
        for j in range(NB):
            if j:
                project_k(j)
                context(2 * j - 2)
                context(2 * j - 1)
            project_v(j)
            parts = diagonal(j)
            if j >= OUT_LAG:
                project_out(j - OUT_LAG)
            scores(2 * j, *parts)
            scores(2 * j + 1, *parts)
        context(2 * NB - 2)
        context(2 * NB - 1)
        for j in range(NB - OUT_LAG, NB):
            project_out(j)
        return carry

    lax.fori_loop(0, H, head_step, 0)
    wait([out_copy(j) for j in range(NB)])


@jax.jit
def pallas_gated_mix__compressed_kv_cla__moe_arch_mod__prompt_kernel(
    A_x: jax.Array,
    A_c_kv: jax.Array,
    A_w_q: jax.Array,
    A_w_uk: jax.Array,
    A_w_uv: jax.Array,
    A_w_o: jax.Array,
    B_x: jax.Array,
    B_w_r: jax.Array,
    B_w_gate: jax.Array,
    B_w_up: jax.Array,
    B_w_down: jax.Array,
    gate_w: jax.Array,
):
    del B_x
    B, S, M = A_x.shape
    _, SK, DC = A_c_kv.shape
    _, H, D = A_w_q.shape
    F = B_w_gate.shape[1]
    assert B == 1 and SK == S
    any_spec = pl.BlockSpec(memory_space=pl.ANY)
    scratch = [
        pltpu.VMEM((1, M // 2, S), U32),
        pltpu.VMEM((S // 2, DC), U32),
        pltpu.VMEM((H // 2, M, D), U32),
        pltpu.VMEM((H // 2, DC, D), U32),
        pltpu.VMEM((H // 2, DC, D), U32),
        pltpu.VMEM((H, M // 2, D), U32),
        pltpu.VMEM((M, F), BF16),
        pltpu.VMEM((M, F), BF16),
        pltpu.VMEM((M, F), BF16),
        pltpu.VMEM((M,), BF16),
        pltpu.VMEM((M,), BF16),
        pltpu.VMEM((7, 1, M), F32),
        pltpu.VMEM((NPQ, D, M), U32),
        pltpu.VMEM((H, D // 2, S), U32),
        pltpu.VMEM((1, S // 2, D), U32),
        pltpu.VMEM((1, D // 2, S), U32),
        [pltpu.VMEM((1, D // 2, TB), U32)] * (S // TB),
        [pltpu.VMEM((1, S, 128), F32)] * 2,
        pltpu.VMEM((M, S), F32),
        pltpu.VMEM((M, S), BF16),
        pltpu.VMEM((8, S), F32),
        pltpu.VMEM((16, M), BF16),
        pltpu.VMEM((16, M), F32),
        pltpu.SMEM((NZ,), I32),
        pltpu.SMEM((2,), I32),
        pltpu.SemaphoreType.DMA((SEM_X + len(X_SPLITS) + 1,)),
    ]
    out_t = pl.pallas_call(
        functools.partial(_kernel, H=H, S=S, D=D, M=M, F=F),
        in_specs=[any_spec] * 11,
        out_specs=any_spec,
        out_shape=jax.ShapeDtypeStruct((M, S), BF16),
        scratch_shapes=scratch,
        compiler_params=pltpu.CompilerParams(
            vmem_limit_bytes=100 * 2**20, internal_scratch_in_bytes=64 * 2**10),
        name="gated_mix",
    )(A_x[0].T, A_c_kv[0], A_w_q, A_w_uk, A_w_uv, jnp.transpose(A_w_o, (0, 2, 1)),
      B_w_r, gate_w, B_w_gate, B_w_up, B_w_down.T)
    return out_t.T[None]
```
